```python
import jax
import jax.numpy as jnp

def _softmax(x, axis=-1):
    return jax.nn.softmax(x, axis=axis)

def _gelu(x):
    return jax.nn.gelu(x, approximate=True)

def _silu(x):
    return jax.nn.silu(x)

def _sigmoid(x):
    return jax.nn.sigmoid(x)

def _layernorm(x, axis=-1, eps=1e-05):
    m = jnp.mean(x, axis=axis, keepdims=True)
    v = jnp.var(x, axis=axis, keepdims=True)
    return (x - m) / jnp.sqrt(v + eps)

def _scatter_add(tgt, idx, src, axis=0):
    return tgt.at[idx].add(src)

def _segment_sum(src, seg, n):
    return jax.ops.segment_sum(src, seg, n)

class _Rng:

    def __init__(self, key):
        self._k = key

    def _next(self):
        self._k, sub = jax.random.split(self._k)
        return sub

    def normal(self, shape):
        return jax.random.normal(self._next(), shape, dtype=jnp.bfloat16)

    def randint(self, lo, hi, shape):
        return jax.random.randint(self._next(), shape, lo, hi, dtype=jnp.int32)

    def uniform(self, shape, lo=0.0, hi=1.0):
        return jax.random.uniform(self._next(), shape, jnp.bfloat16, lo, hi)

    def permutation(self, n):
        return jax.random.permutation(self._next(), n)
kernel_name = 'sequential_preLN__ssm_conv_s4__mixer_gmlp__prompt'

def _fwd_setup_inputs():
    _rng = _Rng(jax.random.key(int.from_bytes(__import__("os").urandom(4), "little")))
    _w = lambda a: (lambda t: t.astype(jnp.bfloat16) if jnp.issubdtype(t.dtype, jnp.floating) else t)(jnp.asarray(a))

    def _A_setup():
        B, L, D, N = (1, 2048, 576, 128)
        A_re = -jnp.exp((lambda *s: _rng.normal(s) * 0.05)(D, N))
        A_im = jnp.pi * (lambda *s: _rng.normal(s) * 0.05)(D, N)
        B_re = (lambda *s: _rng.normal(s) * 0.05)(D, N)
        B_im = (lambda *s: _rng.normal(s) * 0.05)(D, N)
        C_re = (lambda *s: _rng.normal(s) * 0.05)(D, N)
        C_im = (lambda *s: _rng.normal(s) * 0.05)(D, N)
        log_dt = (lambda *s: _rng.normal(s) * 0.05)(D) * 0.5 - 4.0
        Dskip = (lambda *s: _rng.normal(s) * 0.05)(D)
        return {'u': _w((lambda *s: _rng.normal(s) * 0.05)(B, L, D)), 'A_re': _w(A_re), 'A_im': _w(A_im), 'B_re': _w(B_re), 'B_im': _w(B_im), 'C_re': _w(C_re), 'C_im': _w(C_im), 'log_dt': _w(log_dt), 'Dskip': _w(Dskip)}
    _A_in = _A_setup()

    def _B_setup():
        B, S, D, F = (1, 2048, 576, 4608)
        Fh = F // 2
        return {'x': _w((lambda *s: _rng.normal(s) * 0.05)(B, S, D)), 'w_in': _w((lambda *s: _rng.normal(s) * 0.05)(D, 2 * Fh)), 'w_sp': _w(0.01 * (lambda *s: _rng.normal(s) * 0.05)(S, S)), 'b_sp': _w(1.0 + 0.01 * (lambda *s: _rng.normal(s) * 0.05)(S)), 'w_out': _w((lambda *s: _rng.normal(s) * 0.05)(Fh, D))}
    _B_in = _B_setup()
    return {'A_u': _A_in['u'], 'A_A_re': _A_in['A_re'], 'A_A_im': _A_in['A_im'], 'A_B_re': _A_in['B_re'], 'A_B_im': _A_in['B_im'], 'A_C_re': _A_in['C_re'], 'A_C_im': _A_in['C_im'], 'A_log_dt': _A_in['log_dt'], 'A_Dskip': _A_in['Dskip'], 'B_x': _B_in['x'], 'B_w_in': _B_in['w_in'], 'B_w_sp': _B_in['w_sp'], 'B_b_sp': _B_in['b_sp'], 'B_w_out': _B_in['w_out']}

def _fwd_reference(A_u, A_A_re, A_A_im, A_B_re, A_B_im, A_C_re, A_C_im, A_log_dt, A_Dskip, B_x, B_w_in, B_w_sp, B_b_sp, B_w_out):

    def _A_ref(u, A_re, A_im, B_re, B_im, C_re, C_im, log_dt, Dskip):
        Bsz, L, D = u.shape
        dt = jnp.exp(log_dt)[:, None]
        A = A_re + 1j * A_im
        Bc = B_re + 1j * B_im
        Cc = C_re + 1j * C_im
        logdA = dt * A
        dB = dt * Bc
        l = (lambda x, dt: x.astype(dt))(jnp.arange(L), A_re.dtype)
        P = jnp.exp(logdA[:, :, None] * l[None, None, :])
        K = jnp.einsum('dn,dnl,dn->dl', Cc, P, dB).real
        L2 = 2 * L
        Kp = jnp.pad(K, ((0, 0), (0, L)))
        up = (lambda x, *d: x.transpose(*d))(u, 0, 2, 1)
        up = jnp.pad(up, ((0, 0), (0, 0), (0, L)))
        Kf = (lambda x, axes=(-2, -1): jnp.fft.rfft2(x.astype(jnp.float32), axes=axes))(Kp[:, None, :], axes=(-2, -1))
        Uf = (lambda x, axes=(-2, -1): jnp.fft.rfft2(x.astype(jnp.float32), axes=axes))(up[:, :, None, :], axes=(-2, -1))
        Yf = Uf * Kf[None, :, :, :]
        y = (lambda x, s, axes=(-2, -1): jnp.fft.irfft2(x, s=s, axes=axes).astype(jnp.bfloat16))(Yf, (1, L2), axes=(-2, -1))[:, :, 0, :L]
        y = (lambda x, *d: x.transpose(*d))(y, 0, 2, 1) + u * Dskip[None, None, :]
        return y

    def _B_ref(x, w_in, w_sp, b_sp, w_out):
        B, S, D = x.shape
        F = w_in.shape[-1]
        Fh = F // 2
        z = _gelu(jnp.einsum('bsd,df->bsf', x, w_in))
        z1 = z[..., :Fh].copy()
        z2 = _layernorm(z[..., Fh:], axis=-1)
        g = jnp.einsum('ts,bsf->btf', w_sp, z2) + b_sp[None, :, None]
        return jnp.einsum('bsf,fd->bsd', z1 * g, w_out)
    x = A_u
    h = x + _A_ref(_layernorm(x, axis=-1), A_A_re, A_A_im, A_B_re, A_B_im, A_C_re, A_C_im, A_log_dt, A_Dskip)
    h2 = h + _B_ref(_layernorm(h, axis=-1), B_w_in, B_w_sp, B_b_sp, B_w_out)
    return h2

def setup_inputs():
    _inp = _fwd_setup_inputs()
    _gk = jax.random.fold_in(jax.random.key(int.from_bytes(__import__("os").urandom(4), "little")), 2 ** 31 - 1)
    _shapes = [[1, 2048, 576]]
    _dtypes = ['bfloat16']
    _gks = jax.random.split(_gk, len(_shapes))
    _gs = [jax.random.normal(k, s, dtype=jnp.dtype(d)) * 0.05 for k, s, d in zip(_gks, _shapes, _dtypes)]
    _inp['grad_out'] = _gs[0]
    return _inp

def reference(A_u, A_A_re, A_A_im, A_B_re, A_B_im, A_C_re, A_C_im, A_log_dt, A_Dskip, B_w_in, B_w_sp, B_b_sp, B_w_out, B_x, grad_out):
    _const = dict(B_x=B_x)

    def _f(*_d):
        return _fwd_reference(**{'A_u': _d[0], 'A_A_re': _d[1], 'A_A_im': _d[2], 'A_B_re': _d[3], 'A_B_im': _d[4], 'A_C_re': _d[5], 'A_C_im': _d[6], 'A_log_dt': _d[7], 'A_Dskip': _d[8], 'B_w_in': _d[9], 'B_w_sp': _d[10], 'B_b_sp': _d[11], 'B_w_out': _d[12], **_const})
    _out, _vjp = jax.vjp(_f, A_u, A_A_re, A_A_im, A_B_re, A_B_im, A_C_re, A_C_im, A_log_dt, A_Dskip, B_w_in, B_w_sp, B_b_sp, B_w_out)
    _grads = _vjp(grad_out)
    _out0 = jnp.asarray(_out)
    return (_out0, *[jnp.asarray(_g) for _g in _grads])
```

```python
import math
import jax
import jax.numpy as jnp
from jax import lax
import jax.experimental.pallas as pl
import jax.experimental.pallas.tpu as pltpu

L, D, N, F2 = 2048, 576, 128, 2304
F = 2 * F2
T = 256
NB = L // T
TM = 256
KC = 648
IB = 32
f32, bf16 = jnp.float32, jnp.bfloat16
EPS = 1e-5


def _nn(a, b):
    return jnp.dot(a, b, preferred_element_type=f32)


def _nt(a, b):
    return lax.dot_general(a, b, (((1,), (1,)), ((), ())), preferred_element_type=f32)


def _tn(a, b):
    return lax.dot_general(a, b, (((0,), (0,)), ((), ())), preferred_element_type=f32)


_C0 = math.sqrt(2.0 / math.pi)


def _gelu_and_grad(x):
    c3 = 0.044715
    inner = _C0 * (x + c3 * x * x * x)
    th = jnp.tanh(inner)
    g = 0.5 * x * (1.0 + th)
    dg = 0.5 * (1.0 + th) + 0.5 * x * (1.0 - th * th) * (_C0 * (1.0 + 3.0 * c3 * x * x))
    return g, dg


def _ln(x):
    m = jnp.mean(x, axis=-1, keepdims=True)
    xc = x - m
    v = jnp.mean(xc * xc, axis=-1, keepdims=True)
    r = lax.rsqrt(v + EPS)
    return xc * r, r


def _ln_bwd(dy, y, r):
    return (dy - jnp.mean(dy, axis=-1, keepdims=True)
            - y * jnp.mean(dy * y, axis=-1, keepdims=True)) * r


def _cmul(ar, ai, br, bi):
    ar, ai, br, bi = [z.astype(f32) for z in (ar, ai, br, bi)]
    return ar * br - ai * bi, ar * bi + ai * br


def _kernel(x_hbm, are_ref, aim_ref, bre_ref, bim_ref, cre_ref, cim_ref, ldt_ref, dsk_ref,
            win_hbm, wsp_hbm, bsp_ref, wout_hbm, go_hbm,
            out_hbm, dx_hbm, dare_ref, daim_ref, dbre_ref, dbim_ref, dcre_ref, dcim_ref,
            dldt_ref, ddsk_ref, dwin_hbm, dwsp_hbm, dbsp_ref, dwout_hbm,
            wf_s, wft_s, sel_s, up_s, rx_s, kc_s, kf_s, sf_s, dyf_s, h_s, v_s, rh_s,
            zp_s, z2_s, r2_s, dg_s, q_s, pg_s, dh_s, m_s,
            x_ref, win_ref, wsp_ref, wout_ref, go_ref, out_ref, dx_ref, dwin_ref, dwsp_ref,
            dwout_ref, sems, t_s, vt_s, acc_s, car_s):
    cin = [pltpu.make_async_copy(a, b, sems.at[k]) for k, (a, b) in enumerate(
        ((x_hbm, x_ref), (win_hbm, win_ref), (wsp_hbm, wsp_ref), (wout_hbm, wout_ref),
         (go_hbm, go_ref)))]
    cout = [pltpu.make_async_copy(a, b, sems.at[5 + k]) for k, (a, b) in enumerate(
        ((out_ref, out_hbm), (dwout_ref, dwout_hbm), (dwsp_ref, dwsp_hbm), (dwin_ref, dwin_hbm),
         (dx_ref, dx_hbm)))]
    for cp in cin:
        cp.start()
    kk = lax.broadcasted_iota(jnp.int32, (2 * T, 2 * T), 0)
    tt = lax.broadcasted_iota(jnp.int32, (2 * T, 2 * T), 1)

    def dft(kk, tt):
        ph = ((2 * (kk % T) + 1) * tt) % (4 * T)
        ang = ph.astype(f32) * (math.pi / (2 * T))
        return jnp.where(kk < T, jnp.cos(ang), -jnp.sin(ang))
    wf_s[...] = dft(kk, tt).astype(bf16)
    wft_s[...] = (dft(tt, kk) * (1.0 / T)).astype(bf16)

    def lr_of_c(c):
        return jnp.where(c < 256, c, jnp.where(c < 384, 256 + 2 * (c - 256),
                         jnp.where(c < 512, 512 + 4 * (c - 384), 1024 + 8 * (c - 512))))
    for m in range(NB):
        ll = lax.broadcasted_iota(jnp.int32, (T, KC), 0) + m * T
        cc = lax.broadcasted_iota(jnp.int32, (T, KC), 1)
        lrnd = ll.astype(f32).astype(bf16).astype(f32).astype(jnp.int32)
        sel_s[pl.ds(m * T, T), :] = jnp.where(lrnd == lr_of_c(cc), 1.0, 0.0).astype(bf16)

    cin[0].wait()
    up_s[pl.ds(0, T), :] = jnp.zeros((T, D), bf16)

    def ln1(t, c):
        r0 = pl.multiple_of(t * TM, TM)
        u, r = _ln(x_ref[pl.ds(r0, TM), :].astype(f32))
        up_s[pl.ds(T + r0, TM), :] = u.astype(bf16)
        rx_s[pl.ds(r0, TM), :] = jnp.broadcast_to(r, (TM, 128))
        return c
    lax.fori_loop(0, L // TM, ln1, 0)

    dt = jnp.exp(ldt_ref[...].astype(f32)).astype(bf16).astype(f32)
    ii = lax.broadcasted_iota(jnp.int32, (IB, D), 0).astype(f32)
    jj = lax.broadcasted_iota(jnp.int32, (8, D), 0).astype(f32) * float(IB)

    def tables(n):
        ar = dt * are_ref[pl.ds(n, 1), :].astype(f32)
        ai = dt * aim_ref[pl.ds(n, 1), :].astype(f32)
        e = jnp.exp(ar * ii)
        lr_, li_ = e * jnp.cos(ai * ii), e * jnp.sin(ai * ii)
        e = jnp.exp(ar * jj)
        hr_, hi_ = e * jnp.cos(ai * jj), e * jnp.sin(ai * jj)
        blocks = []
        for j in range(8):
            blocks.append((IB * j, lr_, li_, hr_[j:j + 1], hi_[j:j + 1]))
        for o in range(1, 4):
            lr_, li_ = _cmul(lr_, li_, lr_, li_)
            hr_, hi_ = _cmul(hr_, hi_, hr_, hi_)
            for j in range(4, 8):
                blocks.append((256 + 128 * (o - 1) + IB * (j - 4), lr_, li_,
                               hr_[j:j + 1], hi_[j:j + 1]))
        er, ei = _cmul(hr_[4:5], hi_[4:5], hr_[4:5], hi_[4:5])
        return blocks, er, ei

    def gcoef(n):
        br = dt * bre_ref[pl.ds(n, 1), :].astype(f32)
        bi = dt * bim_ref[pl.ds(n, 1), :].astype(f32)
        cr = cre_ref[pl.ds(n, 1), :].astype(f32)
        ci = cim_ref[pl.ds(n, 1), :].astype(f32)
        gr, gi = _cmul(cr, ci, br, bi)
        return gr, gi, br, bi, cr, ci

    kc_s[...] = jnp.zeros((KC, D), f32)

    def kgen(n, c):
        blocks, er, ei = tables(n)
        gr, gi = gcoef(n)[:2]
        for (r0, lr_, li_, hr, hi) in blocks:
            a, b = _cmul(gr, gi, hr, hi)
            kc_s[pl.ds(r0, IB), :] += a * lr_ - b * li_
        kc_s[pl.ds(640, 1), :] += gr * er - gi * ei
        return c
    lax.fori_loop(0, N, kgen, 0)

    def cacc(ar, ai, br, bi, conj):
        ar, ai, br, bi = [z.astype(f32) for z in (ar, ai, br, bi)]
        if conj:
            bi = -bi
        acc_s[0:T, :] += ar * br - ai * bi
        acc_s[T:2 * T, :] += ar * bi + ai * br

    def blk(i):
        return pl.ds(pl.multiple_of(i * T, T), T)

    def f1(m, c):
        km = _nn(sel_s[blk(m), :], kc_s[...].astype(bf16)).astype(bf16)
        kf_s[m] = _nn(wf_s[:, 0:T], km).astype(bf16)
        sf_s[m] = _nn(wf_s[...], up_s[pl.ds(pl.multiple_of(m * T, T), 2 * T), :]).astype(bf16)
        return c
    lax.fori_loop(0, NB, f1, 0)
    dsk = dsk_ref[...].astype(f32)

    def f2(i, c):
        acc_s[...] = jnp.zeros((2 * T, D), f32)

        def g(m, c):
            cacc(kf_s[m, 0:T], kf_s[m, T:2 * T], sf_s[i - m, 0:T], sf_s[i - m, T:2 * T], False)
            return c
        lax.fori_loop(0, i + 1, g, 0)
        y = _nn(wft_s[T:2 * T, :], acc_s[...].astype(bf16)).astype(bf16).astype(f32)
        u = up_s[blk(i + 1), :].astype(f32)
        y = (y + (u * dsk).astype(bf16).astype(f32)).astype(bf16).astype(f32)
        h = (x_ref[blk(i), :].astype(f32) + y).astype(bf16)
        out_ref[blk(i), :] = h
        v, r = _ln(h.astype(f32))
        v_s[blk(i), :] = v.astype(bf16)
        rh_s[blk(i), :] = jnp.broadcast_to(r, (T, 128))
        return c
    lax.fori_loop(0, NB, f2, 0)

    cin[1].wait()
    CW = 256

    def pa(t, c):
        r0 = pl.multiple_of(t * TM, TM)
        rows = pl.ds(r0, TM)
        vt = v_s[rows, :]
        for c0 in range(0, F, 512):
            zp_s[rows, c0:c0 + 512] = _nn(vt, win_ref[:, c0:c0 + 512]).astype(bf16)
        z, _ = _gelu_and_grad(zp_s[rows, F2:F].astype(f32))
        z2, r = _ln(z.astype(bf16).astype(f32))
        z2_s[rows, :] = z2.astype(bf16)
        r2_s[rows, :] = jnp.broadcast_to(r, (TM, 128))
        return c
    lax.fori_loop(0, L // TM, pa, 0)

    cin[2].wait()
    cin[3].wait()
    cin[4].wait()

    def pb(t, c):
        r0 = pl.multiple_of(t * TM, TM)
        rows = pl.ds(r0, TM)
        wt = wsp_ref[rows, :]
        got = go_ref[rows, :]
        bt = bsp_ref[rows, :].astype(f32)
        o = jnp.zeros((TM, D), f32)
        dbs = jnp.zeros((TM, 1), f32)
        for c0 in range(0, F2, CW):
            cs = slice(c0, c0 + CW)
            g = (_nn(wt, z2_s[:, cs]) + bt).astype(bf16).astype(f32)
            z1, dgl = _gelu_and_grad(zp_s[rows, cs].astype(f32))
            z1 = z1.astype(bf16).astype(f32)
            q = (z1 * g).astype(bf16)
            if c0 < L:
                dwsp_ref[rows, cs] = q
            else:
                q_s[rows, :] = q
            o = o + _nn(q, wout_ref[cs, :])
            dq = _nt(got, wout_ref[cs, :]).astype(bf16).astype(f32)
            dgv = dq * z1
            dg_s[rows, cs] = dgv.astype(bf16)
            dbs = dbs + jnp.sum(dgv, axis=-1, keepdims=True)
            zp_s[rows, cs] = (dq * g * dgl).astype(bf16)
        out_ref[rows, :] = (out_ref[rows, :].astype(f32) + o.astype(bf16).astype(f32)).astype(bf16)
        dbsp_ref[rows, :] = dbs.astype(bf16)
        return c
    lax.fori_loop(0, L // TM, pb, 0)
    cout[0].start()

    def pw(t, c):
        c0 = pl.multiple_of(t * 256, 256)
        dwout_ref[pl.ds(c0, 256), :] = _tn(dwsp_ref[:, pl.ds(c0, 256)], go_ref[...]).astype(bf16)
        return c
    lax.fori_loop(0, L // 256, pw, 0)
    dwout_ref[L:F2, :] = _tn(q_s[...], go_ref[...]).astype(bf16)
    cout[1].start()

    def pc(t, c):
        r0 = pl.multiple_of(t * TM, TM)
        rows = pl.ds(r0, TM)
        wT = wsp_ref[:, rows].T
        for c0 in range(0, F2, CW):
            t_s[:, c0:c0 + CW] = _nn(wT, dg_s[:, c0:c0 + CW])
        dzz = _ln_bwd(t_s[...], z2_s[rows, :].astype(f32), r2_s[rows, 0:1])
        _, dgl = _gelu_and_grad(zp_s[rows, F2:F].astype(f32))
        zp_s[rows, F2:F] = (dzz * dgl).astype(bf16)
        dgt = dg_s[rows, :]
        for c0 in range(0, L, CW):
            dwsp_ref[rows, c0:c0 + CW] = _nt(dgt, z2_s[c0:c0 + CW, :]).astype(bf16)
        return c
    lax.fori_loop(0, L // TM, pc, 0)
    cout[2].start()

    def pd(t, c):
        r0 = pl.multiple_of(t * TM, TM)
        rows = pl.ds(r0, TM)
        dv = jnp.zeros((TM, D), f32)
        for c0 in range(0, F, 512):
            dv = dv + _nt(zp_s[rows, c0:c0 + 512], win_ref[:, c0:c0 + 512])
        dh = go_ref[rows, :].astype(f32) + _ln_bwd(dv, v_s[rows, :].astype(f32), rh_s[rows, 0:1])
        dx_ref[rows, :] = dh.astype(bf16)
        vt_s[:, rows] = v_s[rows, :].T
        return c
    lax.fori_loop(0, L // TM, pd, 0)

    def pe(t, c):
        c0 = pl.multiple_of(t * 256, 256)
        dwin_ref[:, pl.ds(c0, 256)] = _nn(vt_s[...], zp_s[:, pl.ds(c0, 256)]).astype(bf16)
        return c
    lax.fori_loop(0, F // 256, pe, 0)
    cout[3].start()

    m_s[...] = jnp.zeros((1, D), f32)

    def b1(i, c):
        dh = dx_ref[blk(i), :]
        dyf_s[i] = _nn(wf_s[:, T:2 * T], dh).astype(bf16)
        m_s[...] += jnp.sum(dh.astype(f32) * up_s[blk(i + 1), :].astype(f32), axis=0, keepdims=True)
        return c
    lax.fori_loop(0, NB, b1, 0)
    ddsk_ref[...] = m_s[...].astype(bf16)
    kc_s[...] = jnp.zeros((KC, D), f32)

    def b2(m, c):
        acc_s[...] = jnp.zeros((2 * T, D), f32)

        def g(i, c):
            cacc(dyf_s[i, 0:T], dyf_s[i, T:2 * T], sf_s[i - m, 0:T], sf_s[i - m, T:2 * T], True)
            return c
        lax.fori_loop(m, NB, g, 0)
        dkm = _nn(wft_s[0:T, :], acc_s[...].astype(bf16)).astype(bf16)
        kc_s[...] += _tn(sel_s[blk(m), :], dkm)
        return c
    lax.fori_loop(0, NB, b2, 0)
    car_s[...] = jnp.zeros((T, D), f32)

    def b3(jr, c):
        j = NB - 1 - jr
        acc_s[...] = jnp.zeros((2 * T, D), f32)

        def g(m, c):
            cacc(dyf_s[j + m, 0:T], dyf_s[j + m, T:2 * T], kf_s[m, 0:T], kf_s[m, T:2 * T], True)
            return c
        lax.fori_loop(0, NB - j, g, 0)
        df = acc_s[...].astype(bf16)
        du = _nn(wft_s[T:2 * T, :], df) + car_s[...]
        car_s[...] = _nn(wft_s[0:T, :], df)
        dh = dx_ref[blk(j), :].astype(f32)
        du = du + dh * dsk
        dx = dh + _ln_bwd(du, up_s[blk(j + 1), :].astype(f32), rx_s[blk(j), 0:1])
        dx_ref[blk(j), :] = dx.astype(bf16)
        return c
    lax.fori_loop(0, NB, b3, 0)

    cout[4].start()
    crow = lax.broadcasted_iota(jnp.int32, (IB, D), 0)

    def fold(a):
        return (a[0:8] + a[8:16]) + (a[16:24] + a[24:32])

    def kbwd(n, c):
        blocks, er, ei = tables(n)
        m0r = jnp.zeros((8, D), f32)
        m0i, m1r, m1i = m0r, m0r, m0r
        for (r0, lr_, li_, hr, hi) in blocks:
            w0 = kc_s[pl.ds(r0, IB), :]
            w1 = w0 * lr_of_c(crow + r0).astype(f32)
            a, b = _cmul(hr, hi, fold(w0 * lr_), fold(w0 * li_))
            m0r, m0i = m0r + a, m0i + b
            a, b = _cmul(hr, hi, fold(w1 * lr_), fold(w1 * li_))
            m1r, m1i = m1r + a, m1i + b
        w = kc_s[pl.ds(640, 1), :]
        red = lambda z: jnp.sum(z, axis=0, keepdims=True)
        m0r, m0i = red(m0r) + w * er, red(m0i) + w * ei
        m1r, m1i = red(m1r) + 2048.0 * w * er, red(m1i) + 2048.0 * w * ei
        gr, gi, br, bi, cr, ci = gcoef(n)
        dgr, dgi = m0r, -m0i
        pr, pi_ = _cmul(gr, gi, m1r, m1i)
        dar, dai = pr, -pi_
        ddbr = dgr * cr + dgi * ci
        ddbi = -dgr * ci + dgi * cr
        row = pl.ds(n, 1)
        pg_s[0, row, :] = (dgr * br + dgi * bi)
        pg_s[1, row, :] = (-dgr * bi + dgi * br)
        pg_s[2, row, :] = (dt * ddbr)
        pg_s[3, row, :] = (dt * ddbi)
        pg_s[4, row, :] = (dt * dar)
        pg_s[5, row, :] = (dt * dai)
        m_s[...] += (ddbr * bre_ref[row, :].astype(f32) + ddbi * bim_ref[row, :].astype(f32)
                     + dar * are_ref[row, :].astype(f32) + dai * aim_ref[row, :].astype(f32))
        return c
    m_s[...] = jnp.zeros((1, D), f32)
    lax.fori_loop(0, N, kbwd, 0)
    dldt_ref[...] = (m_s[...] * dt).astype(bf16)
    for k, r in enumerate((dcre_ref, dcim_ref, dbre_ref, dbim_ref, dare_ref, daim_ref)):
        r[...] = pg_s[k].astype(bf16)
    for cp in cout:
        cp.wait()


@jax.jit
def pallas_sequential_preLN__ssm_conv_s4__mixer_gmlp__prompt_kernel(
        A_u, A_A_re, A_A_im, A_B_re, A_B_im, A_C_re, A_C_im, A_log_dt, A_Dskip,
        B_x, B_w_in, B_w_sp, B_b_sp, B_w_out, grad_out):
    sds = jax.ShapeDtypeStruct
    out_shape = (
        sds((L, D), bf16), sds((L, D), bf16),
        *[sds((N, D), bf16) for _ in range(6)],
        sds((1, D), bf16), sds((1, D), bf16),
        sds((D, F), bf16), sds((L, L), bf16), sds((L, 1), bf16), sds((F2, D), bf16),
    )
    V = pltpu.VMEM
    AN = pl.BlockSpec(memory_space=pl.ANY)
    VM = pl.BlockSpec(memory_space=pltpu.VMEM)
    scratch = [
        V((2 * T, 2 * T), bf16), V((2 * T, 2 * T), bf16), V((L, KC), bf16),
        V((L + T, D), bf16), V((L, 128), f32), V((KC, D), f32),
        V((NB, 2 * T, D), bf16), V((NB, 2 * T, D), bf16), V((NB, 2 * T, D), bf16),
        V((8, D), bf16), V((L, D), bf16), V((L, 128), f32),
        V((L, F), bf16), V((L, F2), bf16), V((L, 128), f32),
        V((L, F2), bf16), V((L, F2 - L), bf16), V((6, N, D), f32),
        V((8, D), bf16), V((1, D), f32),
        V((L, D), bf16), V((D, F), bf16), V((L, L), bf16), V((F2, D), bf16), V((L, D), bf16),
        V((L, D), bf16), V((L, D), bf16), V((D, F), bf16), V((L, L), bf16), V((F2, D), bf16),
        pltpu.SemaphoreType.DMA((10,)), V((TM, F2), f32), V((D, L), bf16), V((2 * T, D), f32), V((T, D), f32),
    ]
    outs = pl.pallas_call(
        _kernel,
        out_shape=out_shape,
        in_specs=[AN] + [VM] * 8 + [AN, AN, VM, AN, AN],
        out_specs=[AN, AN] + [VM] * 8 + [AN, AN, VM, AN],
        scratch_shapes=scratch,
        compiler_params=pltpu.CompilerParams(vmem_limit_bytes=127 * 1024 * 1024),
    )(A_u[0], *[a.T.astype(f32) for a in (A_A_re, A_A_im, A_B_re, A_B_im, A_C_re, A_C_im)],
      A_log_dt.reshape(1, D), A_Dskip.reshape(1, D),
      B_w_in, B_w_sp, B_b_sp.reshape(L, 1), B_w_out, grad_out[0])
    (out, dx, dare, daim, dbre, dbim, dcre, dcim, dldt, ddsk, dwin, dwsp, dbsp, dwout) = outs
    return (out[None], dx[None], dare.T, daim.T, dbre.T, dbim.T, dcre.T, dcim.T,
            dldt.reshape(D), ddsk.reshape(D), dwin, dwsp, dbsp.reshape(L), dwout)
```

```python
import math
import jax
import jax.numpy as jnp
from jax import lax
import jax.experimental.pallas as pl
import jax.experimental.pallas.tpu as pltpu

L, D, N, F2 = 2048, 576, 128, 2304
F = 2 * F2
T = 256
NB = L // T
TM = 256
KC = 648
IB = 32
f32, bf16 = jnp.float32, jnp.bfloat16
EPS = 1e-5


def _nn(a, b):
    return jnp.dot(a, b, preferred_element_type=f32)


def _nt(a, b):
    return lax.dot_general(a, b, (((1,), (1,)), ((), ())), preferred_element_type=f32)


def _tn(a, b):
    return lax.dot_general(a, b, (((0,), (0,)), ((), ())), preferred_element_type=f32)


_C0 = math.sqrt(2.0 / math.pi)


def _gelu_and_grad(x):
    c3 = 0.044715
    inner = _C0 * (x + c3 * x * x * x)
    th = jnp.tanh(inner)
    g = 0.5 * x * (1.0 + th)
    dg = 0.5 * (1.0 + th) + 0.5 * x * (1.0 - th * th) * (_C0 * (1.0 + 3.0 * c3 * x * x))
    return g, dg


def _ln(x):
    m = jnp.mean(x, axis=-1, keepdims=True)
    xc = x - m
    v = jnp.mean(xc * xc, axis=-1, keepdims=True)
    r = lax.rsqrt(v + EPS)
    return xc * r, r


def _ln_bwd(dy, y, r):
    return (dy - jnp.mean(dy, axis=-1, keepdims=True)
            - y * jnp.mean(dy * y, axis=-1, keepdims=True)) * r


def _cmul(ar, ai, br, bi):
    ar, ai, br, bi = [z.astype(f32) for z in (ar, ai, br, bi)]
    return ar * br - ai * bi, ar * bi + ai * br


def _kernel(x_hbm, are_ref, aim_ref, bre_ref, bim_ref, cre_ref, cim_ref, ldt_ref, dsk_ref,
            win_hbm, wsp_hbm, bsp_ref, wout_hbm, go_hbm,
            out_hbm, dx_hbm, dare_ref, daim_ref, dbre_ref, dbim_ref, dcre_ref, dcim_ref,
            dldt_ref, ddsk_ref, dwin_hbm, dwsp_hbm, dbsp_ref, dwout_hbm,
            wf_s, wft_s, sel_s, up_s, rx_s, kc_s, kf_s, sf_s, dyf_s, h_s, v_s, rh_s,
            zp_s, z2_s, r2_s, dg_s, q_s, pg_s, dh_s, m_s,
            x_ref, win_ref, wsp_ref, wout_ref, go_ref, out_ref, dx_ref, dwin_ref, dwsp_ref,
            dwout_ref, sems, t_s, vt_s, acc_s, car_s, kc1_s, pp_s):
    cin = [pltpu.make_async_copy(a, b, sems.at[k]) for k, (a, b) in enumerate(
        ((x_hbm, x_ref), (win_hbm, win_ref), (wsp_hbm, wsp_ref), (wout_hbm, wout_ref),
         (go_hbm, go_ref)))]
    cout = [pltpu.make_async_copy(a, b, sems.at[5 + k]) for k, (a, b) in enumerate(
        ((x_ref, out_hbm), (dwout_ref, dwout_hbm), (dwsp_ref, dwsp_hbm), (dwin_ref, dwin_hbm),
         (vt_s, dx_hbm)))]
    for cp in cin:
        cp.start()
    kk = lax.broadcasted_iota(jnp.int32, (2 * T, 2 * T), 0)
    tt = lax.broadcasted_iota(jnp.int32, (2 * T, 2 * T), 1)

    def dft(kk, tt):
        ph = ((2 * (kk % T) + 1) * tt) % (4 * T)
        ang = ph.astype(f32) * (math.pi / (2 * T))
        return jnp.where(kk < T, jnp.cos(ang), -jnp.sin(ang))
    wf_s[...] = dft(kk, tt).astype(bf16)
    wft_s[...] = (dft(tt, kk) * (1.0 / T)).astype(bf16)

    def lr_of_c(c):
        return jnp.where(c < 256, c, jnp.where(c < 384, 256 + 2 * (c - 256),
                         jnp.where(c < 512, 512 + 4 * (c - 384), 1024 + 8 * (c - 512))))
    for m in range(NB):
        ll = lax.broadcasted_iota(jnp.int32, (T, KC), 0) + m * T
        cc = lax.broadcasted_iota(jnp.int32, (T, KC), 1)
        lrnd = ll.astype(f32).astype(bf16).astype(f32).astype(jnp.int32)
        sel_s[pl.ds(m * T, T), :] = jnp.where(lrnd == lr_of_c(cc), 1.0, 0.0).astype(bf16)

    cin[0].wait()
    up_s[pl.ds(0, T), :] = jnp.zeros((T, D), bf16)

    def ln1(t, c):
        r0 = pl.multiple_of(t * TM, TM)
        u, r = _ln(x_ref[:, pl.ds(r0, TM)].T.astype(f32))
        up_s[pl.ds(T + r0, TM), :] = u.astype(bf16)
        rx_s[pl.ds(r0, TM), 0:1] = r
        return c
    lax.fori_loop(0, L // TM, ln1, 0)

    for k, r in enumerate((are_ref, aim_ref, bre_ref, bim_ref, cre_ref, cim_ref)):
        pp_s[k] = r[...].astype(f32).T
    are_ref, aim_ref, bre_ref, bim_ref, cre_ref, cim_ref = [pp_s.at[k] for k in range(6)]
    dt = jnp.exp(ldt_ref[...].astype(f32)).astype(bf16).astype(f32)
    r8 = lax.broadcasted_iota(jnp.int32, (8, D), 0)
    p2 = lax.shift_left(jnp.ones((8, D), jnp.int32), r8).astype(f32)
    bits = [(lax.shift_right_logical(r8, k) & 1) == 1 for k in range(3)]

    def bittable(er, ei, k0):
        tr = jnp.where(bits[0], er[k0:k0 + 1], 1.0)
        ti = jnp.where(bits[0], ei[k0:k0 + 1], 0.0)
        for k in (1, 2):
            fr = jnp.where(bits[k], er[k0 + k:k0 + k + 1], 1.0)
            fi = jnp.where(bits[k], ei[k0 + k:k0 + k + 1], 0.0)
            tr, ti = _cmul(tr, ti, fr, fi)
        return tr, ti

    def tables(n):
        ar = dt * are_ref[pl.ds(n, 1), :].astype(f32)
        ai = dt * aim_ref[pl.ds(n, 1), :].astype(f32)
        e = jnp.exp(ar * p2)
        er, ei = e * jnp.cos(ai * p2), e * jnp.sin(ai * p2)
        t0r, t0i = bittable(er, ei, 0)
        t1r, t1i = _cmul(t0r, t0i, er[3:4], ei[3:4])
        t2r, t2i = _cmul(t0r, t0i, er[4:5], ei[4:5])
        t3r, t3i = _cmul(t1r, t1i, er[4:5], ei[4:5])
        lr_ = jnp.concatenate([t0r, t1r, t2r, t3r], axis=0)
        li_ = jnp.concatenate([t0i, t1i, t2i, t3i], axis=0)
        hr_, hi_ = bittable(er, ei, 5)
        blocks = []
        for j in range(8):
            blocks.append((IB * j, lr_, li_, hr_[j:j + 1], hi_[j:j + 1]))
        for o in range(1, 4):
            lr_, li_ = _cmul(lr_, li_, lr_, li_)
            hr_, hi_ = _cmul(hr_, hi_, hr_, hi_)
            for j in range(4, 8):
                blocks.append((256 + 128 * (o - 1) + IB * (j - 4), lr_, li_,
                               hr_[j:j + 1], hi_[j:j + 1]))
        er, ei = _cmul(hr_[4:5], hi_[4:5], hr_[4:5], hi_[4:5])
        return blocks, er, ei

    def gcoef(n):
        br = dt * bre_ref[pl.ds(n, 1), :].astype(f32)
        bi = dt * bim_ref[pl.ds(n, 1), :].astype(f32)
        cr = cre_ref[pl.ds(n, 1), :].astype(f32)
        ci = cim_ref[pl.ds(n, 1), :].astype(f32)
        gr, gi = _cmul(cr, ci, br, bi)
        return gr, gi, br, bi, cr, ci

    kc_s[...] = jnp.zeros((KC, D), f32)

    def kgen(n, c):
        blocks, er, ei = tables(n)
        gr, gi = gcoef(n)[:2]
        for (r0, lr_, li_, hr, hi) in blocks:
            a, b = _cmul(gr, gi, hr, hi)
            kc_s[pl.ds(r0, IB), :] += a * lr_ - b * li_
        kc_s[pl.ds(640, 1), :] += gr * er - gi * ei
        return c
    lax.fori_loop(0, N, kgen, 0)

    def cacc(ar, ai, br, bi, conj):
        ar, ai, br, bi = [z.astype(f32) for z in (ar, ai, br, bi)]
        if conj:
            bi = -bi
        acc_s[0:T, :] += ar * br - ai * bi
        acc_s[T:2 * T, :] += ar * bi + ai * br

    def blk(i):
        return pl.ds(pl.multiple_of(i * T, T), T)

    def f1(m, c):
        km = _nn(sel_s[blk(m), :], kc_s[...].astype(bf16)).astype(bf16)
        kf_s[m] = _nn(wf_s[:, 0:T], km).astype(bf16)
        sf_s[m] = _nn(wf_s[...], up_s[pl.ds(pl.multiple_of(m * T, T), 2 * T), :]).astype(bf16)
        return c
    lax.fori_loop(0, NB, f1, 0)
    dsk = dsk_ref[...].astype(f32)

    def f2(i, c):
        acc_s[...] = jnp.zeros((2 * T, D), f32)

        def g(m, c):
            cacc(kf_s[m, 0:T], kf_s[m, T:2 * T], sf_s[i - m, 0:T], sf_s[i - m, T:2 * T], False)
            return c
        lax.fori_loop(0, i + 1, g, 0)
        y = _nn(wft_s[T:2 * T, :], acc_s[...].astype(bf16)).astype(bf16).astype(f32)
        u = up_s[blk(i + 1), :].astype(f32)
        y = (y + (u * dsk).astype(bf16).astype(f32)).astype(bf16).astype(f32)
        h = (x_ref[:, blk(i)].T.astype(f32) + y).astype(bf16)
        out_ref[blk(i), :] = h
        v, r = _ln(h.astype(f32))
        v_s[blk(i), :] = v.astype(bf16)
        rx_s[blk(i), 1:2] = r
        return c
    lax.fori_loop(0, NB, f2, 0)

    cin[1].wait()
    CW = 256

    def pa(t, c):
        r0 = pl.multiple_of(t * TM, TM)
        rows = pl.ds(r0, TM)
        vt = v_s[rows, :]
        for c0 in range(0, F, 512):
            zp_s[rows, c0:c0 + 512] = _nn(vt, win_ref[:, c0:c0 + 512]).astype(bf16)
        z, _ = _gelu_and_grad(zp_s[rows, F2:F].astype(f32))
        z2, r = _ln(z.astype(bf16).astype(f32))
        z2_s[rows, :] = z2.astype(bf16)
        rx_s[rows, 2:3] = r
        return c
    lax.fori_loop(0, L // TM, pa, 0)

    cin[2].wait()
    cin[3].wait()
    cin[4].wait()

    def pb(t, c):
        r0 = pl.multiple_of(t * TM, TM)
        rows = pl.ds(r0, TM)
        wt = wsp_ref[rows, :]
        got = go_ref[:, rows].T
        bt = bsp_ref[rows, :].astype(f32)
        o = jnp.zeros((TM, D), f32)
        dbs = jnp.zeros((TM, 1), f32)
        for c0 in range(0, F2, CW):
            cs = slice(c0, c0 + CW)
            g = (_nn(wt, z2_s[:, cs]) + bt).astype(bf16).astype(f32)
            z1, dgl = _gelu_and_grad(zp_s[rows, cs].astype(f32))
            z1 = z1.astype(bf16).astype(f32)
            q = (z1 * g).astype(bf16)
            if c0 < L:
                dwsp_ref[rows, cs] = q
            else:
                q_s[rows, :] = q
            o = o + _nt(q, wout_ref[:, cs])
            dq = _nn(got, wout_ref[:, cs]).astype(bf16).astype(f32)
            dgv = dq * z1
            dg_s[rows, cs] = dgv.astype(bf16)
            dbs = dbs + jnp.sum(dgv, axis=-1, keepdims=True)
            zp_s[rows, cs] = (dq * g * dgl).astype(bf16)
        x_ref[:, rows] = (out_ref[rows, :].astype(f32) + o.astype(bf16).astype(f32)).astype(bf16).T
        dbsp_ref[rows, :] = dbs.astype(bf16)
        return c
    lax.fori_loop(0, L // TM, pb, 0)
    cout[0].start()

    def pw(t, c):
        c0 = pl.multiple_of(t * 256, 256)
        dwout_ref[:, pl.ds(c0, 256)] = _nn(go_ref[...], dwsp_ref[:, pl.ds(c0, 256)]).astype(bf16)
        return c
    lax.fori_loop(0, L // 256, pw, 0)
    dwout_ref[:, L:F2] = _nn(go_ref[...], q_s[...]).astype(bf16)
    cout[1].start()

    def pc(t, c):
        r0 = pl.multiple_of(t * TM, TM)
        rows = pl.ds(r0, TM)
        wT = wsp_ref[:, rows].T
        for c0 in range(0, F2, CW):
            t_s[:, c0:c0 + CW] = _nn(wT, dg_s[:, c0:c0 + CW])
        dzz = _ln_bwd(t_s[...], z2_s[rows, :].astype(f32), rx_s[rows, 2:3])
        _, dgl = _gelu_and_grad(zp_s[rows, F2:F].astype(f32))
        zp_s[rows, F2:F] = (dzz * dgl).astype(bf16)
        dgt = dg_s[rows, :]
        for c0 in range(0, L, CW):
            dwsp_ref[rows, c0:c0 + CW] = _nt(dgt, z2_s[c0:c0 + CW, :]).astype(bf16)
        return c
    lax.fori_loop(0, L // TM, pc, 0)
    cout[2].start()

    def pd(t, c):
        r0 = pl.multiple_of(t * TM, TM)
        rows = pl.ds(r0, TM)
        dv = jnp.zeros((TM, D), f32)
        for c0 in range(0, F, 512):
            dv = dv + _nt(zp_s[rows, c0:c0 + 512], win_ref[:, c0:c0 + 512])
        dh = go_ref[:, rows].T.astype(f32) + _ln_bwd(dv, v_s[rows, :].astype(f32), rx_s[rows, 1:2])
        dx_ref[rows, :] = dh.astype(bf16)
        vt_s[:, rows] = v_s[rows, :].T
        return c
    lax.fori_loop(0, L // TM, pd, 0)

    def pe(t, c):
        c0 = pl.multiple_of(t * 256, 256)
        dwin_ref[:, pl.ds(c0, 256)] = _nn(vt_s[...], zp_s[:, pl.ds(c0, 256)]).astype(bf16)
        return c
    lax.fori_loop(0, F // 256, pe, 0)
    cout[3].start()

    m_s[...] = jnp.zeros((1, D), f32)

    def b1(i, c):
        dh = dx_ref[blk(i), :]
        dyf_s[i] = _nn(wf_s[:, T:2 * T], dh).astype(bf16)
        m_s[...] += jnp.sum(dh.astype(f32) * up_s[blk(i + 1), :].astype(f32), axis=0, keepdims=True)
        return c
    lax.fori_loop(0, NB, b1, 0)
    ddsk_ref[...] = m_s[...].astype(bf16)
    kc_s[...] = jnp.zeros((KC, D), f32)

    def b2(m, c):
        acc_s[...] = jnp.zeros((2 * T, D), f32)

        def g(i, c):
            cacc(dyf_s[i, 0:T], dyf_s[i, T:2 * T], sf_s[i - m, 0:T], sf_s[i - m, T:2 * T], True)
            return c
        lax.fori_loop(m, NB, g, 0)
        dkm = _nn(wft_s[0:T, :], acc_s[...].astype(bf16)).astype(bf16)
        kc_s[...] += _tn(sel_s[blk(m), :], dkm)
        return c
    lax.fori_loop(0, NB, b2, 0)
    car_s[...] = jnp.zeros((T, D), f32)

    def b3(jr, c):
        j = NB - 1 - jr
        acc_s[...] = jnp.zeros((2 * T, D), f32)

        def g(m, c):
            cacc(dyf_s[j + m, 0:T], dyf_s[j + m, T:2 * T], kf_s[m, 0:T], kf_s[m, T:2 * T], True)
            return c
        lax.fori_loop(0, NB - j, g, 0)
        df = acc_s[...].astype(bf16)
        du = _nn(wft_s[T:2 * T, :], df) + car_s[...]
        car_s[...] = _nn(wft_s[0:T, :], df)
        dh = dx_ref[blk(j), :].astype(f32)
        du = du + dh * dsk
        dx = dh + _ln_bwd(du, up_s[blk(j + 1), :].astype(f32), rx_s[blk(j), 0:1])
        vt_s[:, blk(j)] = dx.astype(bf16).T
        return c
    lax.fori_loop(0, NB, b3, 0)

    cout[4].start()
    kc1_s[...] = kc_s[...] * lr_of_c(lax.broadcasted_iota(jnp.int32, (KC, D), 0)).astype(f32)

    def fold(a):
        return (a[0:8] + a[8:16]) + (a[16:24] + a[24:32])

    def kbwd(n, c):
        blocks, er, ei = tables(n)
        m0r = jnp.zeros((8, D), f32)
        m0i, m1r, m1i = m0r, m0r, m0r
        for bi_, (r0, lr_, li_, hr, hi) in enumerate(blocks):
            w0 = kc_s[pl.ds(r0, IB), :]
            w1 = kc1_s[pl.ds(r0, IB), :]
            a, b = _cmul(hr, hi, fold(w0 * lr_), fold(w0 * li_))
            m0r, m0i = m0r + a, m0i + b
            a, b = _cmul(hr, hi, fold(w1 * lr_), fold(w1 * li_))
            m1r, m1i = m1r + a, m1i + b
        w = kc_s[pl.ds(640, 1), :]
        red = lambda z: jnp.sum(z, axis=0, keepdims=True)
        m0r, m0i = red(m0r) + w * er, red(m0i) + w * ei
        m1r, m1i = red(m1r) + 2048.0 * w * er, red(m1i) + 2048.0 * w * ei
        gr, gi, br, bi, cr, ci = gcoef(n)
        dgr, dgi = m0r, -m0i
        pr, pi_ = _cmul(gr, gi, m1r, m1i)
        dar, dai = pr, -pi_
        ddbr = dgr * cr + dgi * ci
        ddbi = -dgr * ci + dgi * cr
        row = pl.ds(n, 1)
        pg_s[0, row, :] = (dgr * br + dgi * bi)
        pg_s[1, row, :] = (-dgr * bi + dgi * br)
        pg_s[2, row, :] = (dt * ddbr)
        pg_s[3, row, :] = (dt * ddbi)
        pg_s[4, row, :] = (dt * dar)
        pg_s[5, row, :] = (dt * dai)
        m_s[...] += (ddbr * bre_ref[row, :].astype(f32) + ddbi * bim_ref[row, :].astype(f32)
                     + dar * are_ref[row, :].astype(f32) + dai * aim_ref[row, :].astype(f32))
        return c
    m_s[...] = jnp.zeros((1, D), f32)
    lax.fori_loop(0, N, kbwd, 0)
    dldt_ref[...] = (m_s[...] * dt).astype(bf16)
    for k, r in enumerate((dcre_ref, dcim_ref, dbre_ref, dbim_ref, dare_ref, daim_ref)):
        r[...] = pg_s[k].T.astype(bf16)
    for cp in cout:
        cp.wait()


@jax.jit
def pallas_sequential_preLN__ssm_conv_s4__mixer_gmlp__prompt_kernel(
        A_u, A_A_re, A_A_im, A_B_re, A_B_im, A_C_re, A_C_im, A_log_dt, A_Dskip,
        B_x, B_w_in, B_w_sp, B_b_sp, B_w_out, grad_out):
    sds = jax.ShapeDtypeStruct
    out_shape = (
        sds((D, L), bf16), sds((D, L), bf16),
        *[sds((D, N), bf16) for _ in range(6)],
        sds((1, D), bf16), sds((1, D), bf16),
        sds((D, F), bf16), sds((L, L), bf16), sds((L, 1), bf16), sds((D, F2), bf16),
    )
    V = pltpu.VMEM
    AN = pl.BlockSpec(memory_space=pl.ANY)
    VM = pl.BlockSpec(memory_space=pltpu.VMEM)
    scratch = [
        V((2 * T, 2 * T), bf16), V((2 * T, 2 * T), bf16), V((L, KC), bf16),
        V((L + T, D), bf16), V((L, 128), f32), V((KC, D), f32),
        V((NB, 2 * T, D), bf16), V((NB, 2 * T, D), bf16), V((NB, 2 * T, D), bf16),
        V((8, D), bf16), V((L, D), bf16), V((8, 128), f32),
        V((L, F), bf16), V((L, F2), bf16), V((8, 128), f32),
        V((L, F2), bf16), V((L, F2 - L), bf16), V((6, N, D), f32),
        V((8, D), bf16), V((1, D), f32),
        V((D, L), bf16), V((D, F), bf16), V((L, L), bf16), V((D, F2), bf16), V((D, L), bf16),
        V((L, D), bf16), V((L, D), bf16), V((D, F), bf16), V((L, L), bf16), V((D, F2), bf16),
        pltpu.SemaphoreType.DMA((10,)), V((TM, F2), f32), V((D, L), bf16), V((2 * T, D), f32), V((T, D), f32), V((KC, D), f32), V((6, N, D), f32),
    ]
    outs = pl.pallas_call(
        _kernel,
        out_shape=out_shape,
        in_specs=[AN] + [VM] * 8 + [AN, AN, VM, AN, AN],
        out_specs=[AN, AN] + [VM] * 8 + [AN, AN, VM, AN],
        scratch_shapes=scratch,
        compiler_params=pltpu.CompilerParams(vmem_limit_bytes=127 * 1024 * 1024),
    )(A_u[0].T, A_A_re, A_A_im, A_B_re, A_B_im, A_C_re, A_C_im,
      A_log_dt.reshape(1, D), A_Dskip.reshape(1, D),
      B_w_in, B_w_sp, B_b_sp.reshape(L, 1), B_w_out.T, grad_out[0].T)
    (out, dx, dare, daim, dbre, dbim, dcre, dcim, dldt, ddsk, dwin, dwsp, dbsp, dwout) = outs
    return (out.T[None], dx.T[None], dare, daim, dbre, dbim, dcre, dcim,
            dldt.reshape(D), ddsk.reshape(D), dwin, dwsp, dbsp.reshape(L), dwout.T)
```

```python
import math
import jax
import jax.numpy as jnp
from jax import lax
import jax.experimental.pallas as pl
import jax.experimental.pallas.tpu as pltpu

L, D, N, F2 = 2048, 576, 128, 2304
F = 2 * F2
T = 256
NB = L // T
TM = 256
KC = 648
IB = 32
f32, bf16 = jnp.float32, jnp.bfloat16
EPS = 1e-5
W2 = 2 * D
N2 = N // 2


def _nn(a, b):
    return jnp.dot(a, b, preferred_element_type=f32)


def _nt(a, b):
    return lax.dot_general(a, b, (((1,), (1,)), ((), ())), preferred_element_type=f32)


def _tn(a, b):
    return lax.dot_general(a, b, (((0,), (0,)), ((), ())), preferred_element_type=f32)


_C0 = math.sqrt(2.0 / math.pi)


def _gelu_and_grad(x):
    c3 = 0.044715
    inner = _C0 * (x + c3 * x * x * x)
    th = jnp.tanh(inner)
    g = 0.5 * x * (1.0 + th)
    dg = 0.5 * (1.0 + th) + 0.5 * x * (1.0 - th * th) * (_C0 * (1.0 + 3.0 * c3 * x * x))
    return g, dg


def _ln(x):
    m = jnp.mean(x, axis=-1, keepdims=True)
    xc = x - m
    v = jnp.mean(xc * xc, axis=-1, keepdims=True)
    r = lax.rsqrt(v + EPS)
    return xc * r, r


def _ln_bwd(dy, y, r):
    return (dy - jnp.mean(dy, axis=-1, keepdims=True)
            - y * jnp.mean(dy * y, axis=-1, keepdims=True)) * r


def _cmul(ar, ai, br, bi):
    ar, ai, br, bi = [z.astype(f32) for z in (ar, ai, br, bi)]
    return ar * br - ai * bi, ar * bi + ai * br


def _kernel(x_hbm, are_ref, aim_ref, bre_ref, bim_ref, cre_ref, cim_ref, ldt_ref, dsk_ref,
            win_hbm, wsp_hbm, bsp_ref, wout_hbm, go_hbm,
            out_hbm, dx_hbm, dare_ref, daim_ref, dbre_ref, dbim_ref, dcre_ref, dcim_ref,
            dldt_ref, ddsk_ref, dwin_hbm, dwsp_hbm, dbsp_ref, dwout_hbm,
            wf_s, wft_s, sel_s, up_s, rx_s, kc_s, kf_s, sf_s, dyf_s, h_s, v_s, rh_s,
            zp_s, z2_s, r2_s, dg_s, q_s, pg_s, dh_s, m_s,
            x_ref, win_ref, wsp_ref, wout_ref, go_ref, out_ref, dx_ref, dwin_ref, dwsp_ref,
            dwout_ref, sems, t_s, vt_s, acc_s, car_s, kc1_s, pp_s, kcb_s, m2_s):
    cin = [pltpu.make_async_copy(a, b, sems.at[k]) for k, (a, b) in enumerate(
        ((x_hbm, x_ref), (win_hbm, win_ref), (wsp_hbm, wsp_ref), (wout_hbm, wout_ref),
         (go_hbm, go_ref)))]
    cout = [pltpu.make_async_copy(a, b, sems.at[5 + k]) for k, (a, b) in enumerate(
        ((x_ref, out_hbm), (dwout_ref, dwout_hbm), (dwsp_ref, dwsp_hbm), (dwin_ref, dwin_hbm),
         (vt_s, dx_hbm)))]
    for cp in cin:
        cp.start()
    kk = lax.broadcasted_iota(jnp.int32, (2 * T, 2 * T), 0)
    tt = lax.broadcasted_iota(jnp.int32, (2 * T, 2 * T), 1)

    def dft(kk, tt):
        ph = ((2 * (kk % T) + 1) * tt) % (4 * T)
        ang = ph.astype(f32) * (math.pi / (2 * T))
        return jnp.where(kk < T, jnp.cos(ang), -jnp.sin(ang))
    wf_s[...] = dft(kk, tt).astype(bf16)
    wft_s[...] = (dft(tt, kk) * (1.0 / T)).astype(bf16)

    def lr_of_c(c):
        return jnp.where(c < 256, c, jnp.where(c < 384, 256 + 2 * (c - 256),
                         jnp.where(c < 512, 512 + 4 * (c - 384), 1024 + 8 * (c - 512))))
    for m in range(NB):
        ll = lax.broadcasted_iota(jnp.int32, (T, KC), 0) + m * T
        cc = lax.broadcasted_iota(jnp.int32, (T, KC), 1)
        lrnd = ll.astype(f32).astype(bf16).astype(f32).astype(jnp.int32)
        sel_s[pl.ds(m * T, T), :] = jnp.where(lrnd == lr_of_c(cc), 1.0, 0.0).astype(bf16)

    cin[0].wait()
    up_s[pl.ds(0, T), :] = jnp.zeros((T, D), bf16)

    def ln1(t, c):
        r0 = pl.multiple_of(t * TM, TM)
        u, r = _ln(x_ref[:, pl.ds(r0, TM)].T.astype(f32))
        up_s[pl.ds(T + r0, TM), :] = u.astype(bf16)
        rx_s[pl.ds(r0, TM), 0:1] = r
        return c
    lax.fori_loop(0, L // TM, ln1, 0)

    for k, r in enumerate((are_ref, aim_ref, bre_ref, bim_ref, cre_ref, cim_ref)):
        tpk = r[...].astype(f32).T
        pp_s[k, :, 0:D] = tpk[0:N2]
        pp_s[k, :, D:W2] = tpk[N2:N]
    are_ref, aim_ref, bre_ref, bim_ref, cre_ref, cim_ref = [pp_s.at[k] for k in range(6)]
    dt1 = jnp.exp(ldt_ref[...].astype(f32)).astype(bf16).astype(f32)
    dt = jnp.concatenate([dt1, dt1], axis=1)
    r8 = lax.broadcasted_iota(jnp.int32, (8, W2), 0)
    p2 = lax.shift_left(jnp.ones((8, W2), jnp.int32), r8).astype(f32)
    bits = [(lax.shift_right_logical(r8, k) & 1) == 1 for k in range(3)]

    def bittable(er, ei, k0):
        tr = jnp.where(bits[0], er[k0:k0 + 1], 1.0)
        ti = jnp.where(bits[0], ei[k0:k0 + 1], 0.0)
        for k in (1, 2):
            fr = jnp.where(bits[k], er[k0 + k:k0 + k + 1], 1.0)
            fi = jnp.where(bits[k], ei[k0 + k:k0 + k + 1], 0.0)
            tr, ti = _cmul(tr, ti, fr, fi)
        return tr, ti

    def tables(n):
        ar = dt * are_ref[pl.ds(n, 1), :].astype(f32)
        ai = dt * aim_ref[pl.ds(n, 1), :].astype(f32)
        e = jnp.exp(ar * p2)
        er, ei = e * jnp.cos(ai * p2), e * jnp.sin(ai * p2)
        t0r, t0i = bittable(er, ei, 0)
        t1r, t1i = _cmul(t0r, t0i, er[3:4], ei[3:4])
        t2r, t2i = _cmul(t0r, t0i, er[4:5], ei[4:5])
        t3r, t3i = _cmul(t1r, t1i, er[4:5], ei[4:5])
        lr_ = jnp.concatenate([t0r, t1r, t2r, t3r], axis=0)
        li_ = jnp.concatenate([t0i, t1i, t2i, t3i], axis=0)
        hr_, hi_ = bittable(er, ei, 5)
        blocks = []
        for j in range(8):
            blocks.append((IB * j, lr_, li_, hr_[j:j + 1], hi_[j:j + 1]))
        for o in range(1, 4):
            lr_, li_ = _cmul(lr_, li_, lr_, li_)
            hr_, hi_ = _cmul(hr_, hi_, hr_, hi_)
            for j in range(4, 8):
                blocks.append((256 + 128 * (o - 1) + IB * (j - 4), lr_, li_,
                               hr_[j:j + 1], hi_[j:j + 1]))
        er, ei = _cmul(hr_[4:5], hi_[4:5], hr_[4:5], hi_[4:5])
        return blocks, er, ei

    def gcoef(n):
        br = dt * bre_ref[pl.ds(n, 1), :].astype(f32)
        bi = dt * bim_ref[pl.ds(n, 1), :].astype(f32)
        cr = cre_ref[pl.ds(n, 1), :].astype(f32)
        ci = cim_ref[pl.ds(n, 1), :].astype(f32)
        gr, gi = _cmul(cr, ci, br, bi)
        return gr, gi, br, bi, cr, ci

    kc_s[...] = jnp.zeros((KC, W2), f32)

    def kgen(n, c):
        blocks, er, ei = tables(n)
        gr, gi = gcoef(n)[:2]
        for (r0, lr_, li_, hr, hi) in blocks:
            a, b = _cmul(gr, gi, hr, hi)
            kc_s[pl.ds(r0, IB), :] += a * lr_ - b * li_
        kc_s[pl.ds(640, 1), :] += gr * er - gi * ei
        return c
    lax.fori_loop(0, N2, kgen, 0)
    kcb_s[...] = (kc_s[:, 0:D] + kc_s[:, D:W2]).astype(bf16)

    def cacc(ar, ai, br, bi, conj):
        ar, ai, br, bi = [z.astype(f32) for z in (ar, ai, br, bi)]
        if conj:
            bi = -bi
        acc_s[0:T, :] += ar * br - ai * bi
        acc_s[T:2 * T, :] += ar * bi + ai * br

    def blk(i):
        return pl.ds(pl.multiple_of(i * T, T), T)

    def f1(m, c):
        km = _nn(sel_s[blk(m), :], kcb_s[...]).astype(bf16)
        kf_s[m] = _nn(wf_s[:, 0:T], km).astype(bf16)
        sf_s[m] = _nn(wf_s[...], up_s[pl.ds(pl.multiple_of(m * T, T), 2 * T), :]).astype(bf16)
        return c
    lax.fori_loop(0, NB, f1, 0)
    dsk = dsk_ref[...].astype(f32)

    def f2(i, c):
        acc_s[...] = jnp.zeros((2 * T, D), f32)

        def g(m, c):
            cacc(kf_s[m, 0:T], kf_s[m, T:2 * T], sf_s[i - m, 0:T], sf_s[i - m, T:2 * T], False)
            return c
        lax.fori_loop(0, i + 1, g, 0)
        y = _nn(wft_s[T:2 * T, :], acc_s[...].astype(bf16)).astype(bf16).astype(f32)
        u = up_s[blk(i + 1), :].astype(f32)
        y = (y + (u * dsk).astype(bf16).astype(f32)).astype(bf16).astype(f32)
        h = (x_ref[:, blk(i)].T.astype(f32) + y).astype(bf16)
        out_ref[blk(i), :] = h
        v, r = _ln(h.astype(f32))
        v_s[blk(i), :] = v.astype(bf16)
        rx_s[blk(i), 1:2] = r
        return c
    lax.fori_loop(0, NB, f2, 0)

    cin[1].wait()
    CW = 256

    def pa(t, c):
        r0 = pl.multiple_of(t * TM, TM)
        rows = pl.ds(r0, TM)
        vt = v_s[rows, :]
        for c0 in range(0, F, 512):
            zp_s[rows, c0:c0 + 512] = _nn(vt, win_ref[:, c0:c0 + 512]).astype(bf16)
        z, _ = _gelu_and_grad(zp_s[rows, F2:F].astype(f32))
        z2, r = _ln(z.astype(bf16).astype(f32))
        z2_s[rows, :] = z2.astype(bf16)
        rx_s[rows, 2:3] = r
        return c
    lax.fori_loop(0, L // TM, pa, 0)

    cin[2].wait()
    cin[3].wait()
    cin[4].wait()

    def pb(t, c):
        r0 = pl.multiple_of(t * TM, TM)
        rows = pl.ds(r0, TM)
        wt = wsp_ref[rows, :]
        got = go_ref[:, rows].T
        bt = bsp_ref[rows, :].astype(f32)
        o = jnp.zeros((TM, D), f32)
        dbs = jnp.zeros((TM, 1), f32)
        for c0 in range(0, F2, CW):
            cs = slice(c0, c0 + CW)
            g = (_nn(wt, z2_s[:, cs]) + bt).astype(bf16).astype(f32)
            z1, dgl = _gelu_and_grad(zp_s[rows, cs].astype(f32))
            z1 = z1.astype(bf16).astype(f32)
            q = (z1 * g).astype(bf16)
            if c0 < L:
                dwsp_ref[rows, cs] = q
            else:
                q_s[rows, :] = q
            o = o + _nt(q, wout_ref[:, cs])
            dq = _nn(got, wout_ref[:, cs]).astype(bf16).astype(f32)
            dgv = dq * z1
            dg_s[rows, cs] = dgv.astype(bf16)
            dbs = dbs + jnp.sum(dgv, axis=-1, keepdims=True)
            zp_s[rows, cs] = (dq * g * dgl).astype(bf16)
        x_ref[:, rows] = (out_ref[rows, :].astype(f32) + o.astype(bf16).astype(f32)).astype(bf16).T
        dbsp_ref[rows, :] = dbs.astype(bf16)
        return c
    lax.fori_loop(0, L // TM, pb, 0)
    cout[0].start()

    def pw(t, c):
        c0 = pl.multiple_of(t * 256, 256)
        dwout_ref[:, pl.ds(c0, 256)] = _nn(go_ref[...], dwsp_ref[:, pl.ds(c0, 256)]).astype(bf16)
        return c
    lax.fori_loop(0, L // 256, pw, 0)
    dwout_ref[:, L:F2] = _nn(go_ref[...], q_s[...]).astype(bf16)
    cout[1].start()

    def pc(t, c):
        r0 = pl.multiple_of(t * TM, TM)
        rows = pl.ds(r0, TM)
        wT = wsp_ref[:, rows].T
        for c0 in range(0, F2, CW):
            t_s[:, c0:c0 + CW] = _nn(wT, dg_s[:, c0:c0 + CW])
        dzz = _ln_bwd(t_s[...], z2_s[rows, :].astype(f32), rx_s[rows, 2:3])
        _, dgl = _gelu_and_grad(zp_s[rows, F2:F].astype(f32))
        zp_s[rows, F2:F] = (dzz * dgl).astype(bf16)
        dgt = dg_s[rows, :]
        for c0 in range(0, L, CW):
            dwsp_ref[rows, c0:c0 + CW] = _nt(dgt, z2_s[c0:c0 + CW, :]).astype(bf16)
        return c
    lax.fori_loop(0, L // TM, pc, 0)
    cout[2].start()

    def pd(t, c):
        r0 = pl.multiple_of(t * TM, TM)
        rows = pl.ds(r0, TM)
        dv = jnp.zeros((TM, D), f32)
        for c0 in range(0, F, 512):
            dv = dv + _nt(zp_s[rows, c0:c0 + 512], win_ref[:, c0:c0 + 512])
        dh = go_ref[:, rows].T.astype(f32) + _ln_bwd(dv, v_s[rows, :].astype(f32), rx_s[rows, 1:2])
        out_ref[rows, :] = dh.astype(bf16)
        vt_s[:, rows] = v_s[rows, :].T
        return c
    lax.fori_loop(0, L // TM, pd, 0)

    def pe(t, c):
        c0 = pl.multiple_of(t * 256, 256)
        dwin_ref[:, pl.ds(c0, 256)] = _nn(vt_s[...], zp_s[:, pl.ds(c0, 256)]).astype(bf16)
        return c
    lax.fori_loop(0, F // 256, pe, 0)
    cout[3].start()

    m_s[...] = jnp.zeros((1, D), f32)

    def b1(i, c):
        dh = out_ref[blk(i), :]
        dyf_s[i] = _nn(wf_s[:, T:2 * T], dh).astype(bf16)
        m_s[...] += jnp.sum(dh.astype(f32) * up_s[blk(i + 1), :].astype(f32), axis=0, keepdims=True)
        return c
    lax.fori_loop(0, NB, b1, 0)
    ddsk_ref[...] = m_s[...].astype(bf16)
    kc_s[:, 0:D] = jnp.zeros((KC, D), f32)

    def b2(m, c):
        acc_s[...] = jnp.zeros((2 * T, D), f32)

        def g(i, c):
            cacc(dyf_s[i, 0:T], dyf_s[i, T:2 * T], sf_s[i - m, 0:T], sf_s[i - m, T:2 * T], True)
            return c
        lax.fori_loop(m, NB, g, 0)
        dkm = _nn(wft_s[0:T, :], acc_s[...].astype(bf16)).astype(bf16)
        kc_s[:, 0:D] += _tn(sel_s[blk(m), :], dkm)
        return c
    lax.fori_loop(0, NB, b2, 0)
    car_s[...] = jnp.zeros((T, D), f32)

    def b3(jr, c):
        j = NB - 1 - jr
        acc_s[...] = jnp.zeros((2 * T, D), f32)

        def g(m, c):
            cacc(dyf_s[j + m, 0:T], dyf_s[j + m, T:2 * T], kf_s[m, 0:T], kf_s[m, T:2 * T], True)
            return c
        lax.fori_loop(0, NB - j, g, 0)
        df = acc_s[...].astype(bf16)
        du = _nn(wft_s[T:2 * T, :], df) + car_s[...]
        car_s[...] = _nn(wft_s[0:T, :], df)
        dh = out_ref[blk(j), :].astype(f32)
        du = du + dh * dsk
        dx = dh + _ln_bwd(du, up_s[blk(j + 1), :].astype(f32), rx_s[blk(j), 0:1])
        vt_s[:, blk(j)] = dx.astype(bf16).T
        return c
    lax.fori_loop(0, NB, b3, 0)

    cout[4].start()
    kc_s[:, D:W2] = kc_s[:, 0:D]
    kc1_s[...] = kc_s[...] * lr_of_c(lax.broadcasted_iota(jnp.int32, (KC, W2), 0)).astype(f32)

    def fold(a):
        return (a[0:8] + a[8:16]) + (a[16:24] + a[24:32])

    def kbwd(n, c):
        blocks, er, ei = tables(n)
        m0r = jnp.zeros((8, W2), f32)
        m0i, m1r, m1i = m0r, m0r, m0r
        for bi_, (r0, lr_, li_, hr, hi) in enumerate(blocks):
            w0 = kc_s[pl.ds(r0, IB), :]
            w1 = kc1_s[pl.ds(r0, IB), :]
            a, b = _cmul(hr, hi, fold(w0 * lr_), fold(w0 * li_))
            m0r, m0i = m0r + a, m0i + b
            a, b = _cmul(hr, hi, fold(w1 * lr_), fold(w1 * li_))
            m1r, m1i = m1r + a, m1i + b
        w = kc_s[pl.ds(640, 1), :]
        red = lambda z: jnp.sum(z, axis=0, keepdims=True)
        m0r, m0i = red(m0r) + w * er, red(m0i) + w * ei
        m1r, m1i = red(m1r) + 2048.0 * w * er, red(m1i) + 2048.0 * w * ei
        gr, gi, br, bi, cr, ci = gcoef(n)
        dgr, dgi = m0r, -m0i
        pr, pi_ = _cmul(gr, gi, m1r, m1i)
        dar, dai = pr, -pi_
        ddbr = dgr * cr + dgi * ci
        ddbi = -dgr * ci + dgi * cr
        row = pl.ds(n, 1)
        pg_s[0, row, :] = (dgr * br + dgi * bi)
        pg_s[1, row, :] = (-dgr * bi + dgi * br)
        pg_s[2, row, :] = (dt * ddbr)
        pg_s[3, row, :] = (dt * ddbi)
        pg_s[4, row, :] = (dt * dar)
        pg_s[5, row, :] = (dt * dai)
        m2_s[...] += (ddbr * bre_ref[row, :].astype(f32) + ddbi * bim_ref[row, :].astype(f32)
                     + dar * are_ref[row, :].astype(f32) + dai * aim_ref[row, :].astype(f32))
        return c
    m2_s[...] = jnp.zeros((1, W2), f32)
    lax.fori_loop(0, N2, kbwd, 0)
    dldt_ref[...] = ((m2_s[:, 0:D] + m2_s[:, D:W2]) * dt1).astype(bf16)
    for k, r in enumerate((dcre_ref, dcim_ref, dbre_ref, dbim_ref, dare_ref, daim_ref)):
        r[...] = jnp.concatenate([pg_s[k, :, 0:D], pg_s[k, :, D:W2]], axis=0).T.astype(bf16)
    for cp in cout:
        cp.wait()


@jax.jit
def pallas_sequential_preLN__ssm_conv_s4__mixer_gmlp__prompt_kernel(
        A_u, A_A_re, A_A_im, A_B_re, A_B_im, A_C_re, A_C_im, A_log_dt, A_Dskip,
        B_x, B_w_in, B_w_sp, B_b_sp, B_w_out, grad_out):
    sds = jax.ShapeDtypeStruct
    out_shape = (
        sds((D, L), bf16), sds((D, L), bf16),
        *[sds((D, N), bf16) for _ in range(6)],
        sds((1, D), bf16), sds((1, D), bf16),
        sds((D, F), bf16), sds((L, L), bf16), sds((L, 1), bf16), sds((D, F2), bf16),
    )
    V = pltpu.VMEM
    AN = pl.BlockSpec(memory_space=pl.ANY)
    VM = pl.BlockSpec(memory_space=pltpu.VMEM)
    scratch = [
        V((2 * T, 2 * T), bf16), V((2 * T, 2 * T), bf16), V((L, KC), bf16),
        V((L + T, D), bf16), V((L, 128), f32), V((KC, W2), f32),
        V((NB, 2 * T, D), bf16), V((NB, 2 * T, D), bf16), V((NB, 2 * T, D), bf16),
        V((8, D), bf16), V((L, D), bf16), V((8, 128), f32),
        V((L, F), bf16), V((L, F2), bf16), V((8, 128), f32),
        V((L, F2), bf16), V((L, F2 - L), bf16), V((6, N2, W2), f32),
        V((8, D), bf16), V((1, D), f32),
        V((D, L), bf16), V((D, F), bf16), V((L, L), bf16), V((D, F2), bf16), V((D, L), bf16),
        V((L, D), bf16), V((16, D), bf16), V((D, F), bf16), V((L, L), bf16), V((D, F2), bf16),
        pltpu.SemaphoreType.DMA((10,)), V((TM, F2), f32), V((D, L), bf16), V((2 * T, D), f32), V((T, D), f32), V((KC, W2), f32), V((6, N2, W2), f32), V((KC, D), bf16), V((1, W2), f32),
    ]
    outs = pl.pallas_call(
        _kernel,
        out_shape=out_shape,
        in_specs=[AN] + [VM] * 8 + [AN, AN, VM, AN, AN],
        out_specs=[AN, AN] + [VM] * 8 + [AN, AN, VM, AN],
        scratch_shapes=scratch,
        compiler_params=pltpu.CompilerParams(vmem_limit_bytes=127 * 1024 * 1024),
    )(A_u[0].T, A_A_re, A_A_im, A_B_re, A_B_im, A_C_re, A_C_im,
      A_log_dt.reshape(1, D), A_Dskip.reshape(1, D),
      B_w_in, B_w_sp, B_b_sp.reshape(L, 1), B_w_out.T, grad_out[0].T)
    (out, dx, dare, daim, dbre, dbim, dcre, dcim, dldt, ddsk, dwin, dwsp, dbsp, dwout) = outs
    return (out.T[None], dx.T[None], dare, daim, dbre, dbim, dcre, dcim,
            dldt.reshape(D), ddsk.reshape(D), dwin, dwsp, dbsp.reshape(L), dwout.T)
```
